```python
import jax
import jax.numpy as jnp

def _softmax(x, axis=-1):
    return jax.nn.softmax(x, axis=axis)
def _gelu(x):
    return jax.nn.gelu(x, approximate=True)
def _silu(x):
    return jax.nn.silu(x)
def _sigmoid(x):
    return jax.nn.sigmoid(x)
def _layernorm(x, axis=-1, eps=1e-5):
    m = jnp.mean(x, axis=axis, keepdims=True)
    v = jnp.var(x, axis=axis, keepdims=True)
    return (x - m) / jnp.sqrt(v + eps)
def _scatter_add(tgt, idx, src, axis=0):
    return tgt.at[idx].add(src)
def _segment_sum(src, seg, n):
    return jax.ops.segment_sum(src, seg, n)
class _Rng:
    def __init__(self, key):
        self._k = key
    def _next(self):
        self._k, sub = jax.random.split(self._k)
        return sub
    def normal(self, shape):
        return jax.random.normal(self._next(), shape, dtype=jnp.bfloat16)
    def randint(self, lo, hi, shape):
        return jax.random.randint(self._next(), shape, lo, hi, dtype=jnp.int32)
    def uniform(self, shape, lo=0.0, hi=1.0):
        return jax.random.uniform(self._next(), shape, jnp.bfloat16, lo, hi)
    def permutation(self, n):
        return jax.random.permutation(self._next(), n)


kernel_name = 'sequential_preLN__grouped_kv_mqa__glu_gated_swiglu__prompt'

def _fwd_setup_inputs():
    _rng = _Rng(jax.random.key(int.from_bytes(__import__("os").urandom(4), "little")))
    _w = (lambda a: (lambda t: t.astype(jnp.bfloat16) if jnp.issubdtype(t.dtype, jnp.floating) else t)(jnp.asarray(a)))
    def _A_setup():
        B, S, D, H = 1, 2048, 512, 32
        Dh = D // H
        return {
            "x": _w((lambda *s: _rng.normal(s) * 0.05)(B, S, D)),
            "wq": _w((lambda *s: _rng.normal(s) * 0.05)(D, H * Dh)),
            "wk": _w((lambda *s: _rng.normal(s) * 0.05)(D, Dh)),
            "wv": _w((lambda *s: _rng.normal(s) * 0.05)(D, Dh)),
            "wo": _w((lambda *s: _rng.normal(s) * 0.05)(H * Dh, D)),
        }
    _A_in = _A_setup()

    def _B_setup():
        B, S, D, F = 1, 2048, 512, 1376
        return {
            "x": _w((lambda *s: _rng.normal(s) * 0.05)(B, S, D)),
            "w1": _w((lambda *s: _rng.normal(s) * 0.05)(D, F) * (2.0 / D) ** 0.5),
            "w3": _w((lambda *s: _rng.normal(s) * 0.05)(D, F) * (2.0 / D) ** 0.5),
            "w2": _w((lambda *s: _rng.normal(s) * 0.05)(F, D) * (2.0 / F) ** 0.5),
        }
    _B_in = _B_setup()

    return {
        "A_x": _A_in["x"],
        "A_wq": _A_in["wq"],
        "A_wk": _A_in["wk"],
        "A_wv": _A_in["wv"],
        "A_wo": _A_in["wo"],
        "B_x": _B_in["x"],
        "B_w1": _B_in["w1"],
        "B_w3": _B_in["w3"],
        "B_w2": _B_in["w2"],
    }

def _fwd_reference(A_x, A_wq, A_wk, A_wv, A_wo, B_x, B_w1, B_w3, B_w2):
    def _A_ref(x, wq, wk, wv, wo):
        B, S, D = x.shape
        H = 32
        Dh = D // H
        q = (lambda x, *d: x.transpose(*d))((x @ wq).reshape(B, S, H, Dh), 0, 2, 1, 3)
        k = x @ wk
        v = x @ wv
        scores = jnp.einsum("bhqd,bkd->bhqk", q, k) * (Dh ** -0.5)
        p = _softmax(scores, axis=-1)
        o = jnp.einsum("bhqk,bkd->bhqd", p, v)
        return (lambda x, *d: x.transpose(*d))(o, 0, 2, 1, 3).reshape(B, S, H * Dh) @ wo

    def _B_ref(x, w1, w3, w2):
        gate = jnp.einsum("bsd,df->bsf", x, w1)
        up = jnp.einsum("bsd,df->bsf", x, w3)
        h = _silu(gate) * up
        out = jnp.einsum("bsf,fd->bsd", h, w2)
        return out

    x = A_x
    h = x + _A_ref(_layernorm(x, axis=-1), A_wq, A_wk, A_wv, A_wo)
    h2 = h + _B_ref(_layernorm(h, axis=-1), B_w1, B_w3, B_w2)
    return h2


def setup_inputs():
    _inp = _fwd_setup_inputs()
    _gk = jax.random.fold_in(jax.random.key(int.from_bytes(__import__("os").urandom(4), "little")), 2**31 - 1)
    _shapes = [[1, 2048, 512]]
    _dtypes = ['bfloat16']
    _gks = jax.random.split(_gk, len(_shapes))
    _gs = [jax.random.normal(k, s, dtype=jnp.dtype(d)) * 0.05 for k, s, d in zip(_gks, _shapes, _dtypes)]
    _inp["grad_out"] = _gs[0]
    return _inp

def reference(A_x, A_wq, A_wk, A_wv, A_wo, B_w1, B_w3, B_w2, B_x, grad_out):
    _const = dict(B_x=B_x)
    def _f(*_d):
        return _fwd_reference(**{'A_x': _d[0], 'A_wq': _d[1], 'A_wk': _d[2], 'A_wv': _d[3], 'A_wo': _d[4], 'B_w1': _d[5], 'B_w3': _d[6], 'B_w2': _d[7], **_const})
    _out, _vjp = jax.vjp(_f, A_x, A_wq, A_wk, A_wv, A_wo, B_w1, B_w3, B_w2)
    _grads = _vjp(grad_out)
    _out0 = jnp.asarray(_out)
    return (_out0, *[jnp.asarray(_g) for _g in _grads])
```

```python
import jax
import jax.numpy as jnp
from jax import lax
import jax.experimental.pallas as pl
import jax.experimental.pallas.tpu as pltpu

S, D, H, DH, F = 2048, 512, 32, 16, 1376
TQ = 128
NB = S // TQ
OC = 128
NC = S // OC
EPS = 1e-5
LOG2E = 1.4426950408889634
SCALE = DH ** -0.5
bf16 = jnp.bfloat16
f32 = jnp.float32
u32 = jnp.uint32
NN = (((1,), (0,)), ((), ()))
NT = (((1,), (1,)), ((), ()))

U = 4
LRS, LRD = 64, 64
SKEW_P, SKEW_K = 4, 4
ORDER = "SDVKPQ"


def dot(a, b, dn=NN):
    return lax.dot_general(a, b, dn, preferred_element_type=f32)


def as_u32(x):
    return pltpu.bitcast(x, u32)


def as_bf16(x):
    return pltpu.bitcast(x, bf16)


def ln_stats(xT):
    mu = jnp.mean(xT, axis=0, keepdims=True)
    xc = xT - mu
    var = jnp.mean(xc * xc, axis=0, keepdims=True)
    rstd = 1.0 / jnp.sqrt(var + EPS)
    return xc * rstd, rstd


def ln_bwd(dxn, xn, rstd):
    m1 = jnp.mean(dxn, axis=0, keepdims=True)
    m2 = jnp.mean(dxn * xn, axis=0, keepdims=True)
    return rstd * (dxn - m1 - xn * m2)


def hs(h):
    return pl.ds(pl.multiple_of(h * DH, DH), DH)


def attention(fwd, bwd, k_s, v_s, kT_s, vT_s, qF, qB, doT_s, delta_s, pF, pB, mF, mB,
              finF, finB, oT_s, dqT_s, dk_acc, dv_acc):
    def lhs(ref, r0, n):
        return as_bf16(ref[r0 // 2:(r0 + n) // 2, :])

    def tT(ref, c):
        return as_bf16(ref[:, c * OC:(c + 1) * OC])

    def cr(c):
        return slice(c * OC, (c + 1) * OC)

    def long_dot(ref, c, w, lr):
        parts = [dot(lhs(ref, c * OC + j * lr, lr), w) for j in range(OC // lr)]
        return parts[0] if len(parts) == 1 else jnp.concatenate(parts, axis=0)

    def block(i, carry):
        hh = [i * U + u for u in range(U)]
        st = [dict(alpha={}, ds={}, w={}) for _ in hh]
        for u, h in enumerate(hh):
            s_ = st[u]
            if fwd:
                s_["q"] = qF[hs(h), :]
                s_["m"] = jnp.full((1, TQ), -1e30, f32)
                s_["l"] = jnp.zeros((8, TQ), f32)
                s_["o"] = jnp.zeros((DH, TQ), f32)
            if bwd:
                s_["qb"] = qB[hs(h), :]
                s_["do"] = doT_s[hs(h), :]
                s_["delta"] = delta_s[h]
                s_["mfin"] = finB[h, 0]
                s_["linv"] = finB[h, 1]
                s_["dq"] = jnp.zeros((DH, TQ), f32)
        T = U * NC

        def S_(t):
            u, c = divmod(t, NC)
            s_ = st[u]
            s = long_dot(k_s, c, s_["q"], LRS)
            mn = jnp.maximum(s_["m"], jnp.max(s, axis=0, keepdims=True))
            p = jnp.exp2(s - mn)
            al = jnp.exp2(s_["m"] - mn)
            s_["l"] = s_["l"] * al + p.reshape(OC // 8, 8, TQ).sum(axis=0)
            pF[hh[u], cr(c), :] = p.astype(bf16)
            mF[hh[u], c] = jnp.broadcast_to(mn, (8, TQ))
            s_["m"] = mn
            s_["alpha"][c] = al

        def P_(t):
            u, c = divmod(t, NC)
            s_ = st[u]
            s_["o"] = s_["o"] * s_["alpha"].pop(c) + dot(tT(vT_s, c), pF[hh[u], cr(c), :])
            if c == NC - 1:
                linv = 1.0 / jnp.sum(s_["l"], axis=0, keepdims=True)
                oT_s[hs(hh[u]), :] = s_["o"] * linv
                finF[hh[u], 0] = jnp.broadcast_to(s_["m"], (8, TQ))
                finF[hh[u], 1] = jnp.broadcast_to(linv, (8, TQ))

        def W_(u, c):
            s_ = st[u]
            if c not in s_["w"]:
                corr = jnp.exp2(mB[hh[u], c] - s_["mfin"]) * s_["linv"]
                w = (s_["do"].reshape(2, 8, TQ) * corr).reshape(DH, TQ).astype(bf16)
                s_["w"][c] = (w, (s_["delta"] * corr)[0:1, :])
            return s_["w"][c]

        def D_(t):
            u, c = divmod(t, NC)
            w, dl = W_(u, c)
            dp = long_dot(v_s, c, w, LRD)
            st[u]["ds"][c] = (pB[hh[u], cr(c), :].astype(f32) * (dp - dl)).astype(bf16)

        def V_(t):
            u, c = divmod(t, NC)
            dv_acc[:, cr(c)] += dot(W_(u, c)[0], pB[hh[u], cr(c), :], NT)

        def K_(t):
            u, c = divmod(t, NC)
            dk_acc[:, cr(c)] += dot(st[u]["qb"], st[u]["ds"][c], NT)

        def Q_(t):
            u, c = divmod(t, NC)
            s_ = st[u]
            s_["dq"] = s_["dq"] + dot(tT(kT_s, c), s_["ds"].pop(c))
            if c == NC - 1:
                dqT_s[hs(hh[u]), :] = s_["dq"]

        for t in range(T + max(SKEW_P, SKEW_K)):
            for op in ORDER:
                if op == "S" and fwd and t < T:
                    S_(t)
                if op == "P" and fwd and 0 <= t - SKEW_P < T:
                    P_(t - SKEW_P)
                if op == "D" and bwd and t < T:
                    D_(t)
                if op == "V" and bwd and t < T:
                    V_(t)
                if op == "K" and bwd and 0 <= t - SKEW_K < T:
                    K_(t - SKEW_K)
                if op == "Q" and bwd and 0 <= t - SKEW_K < T:
                    Q_(t - SKEW_K)
        return carry

    lax.fori_loop(0, H // U, block, 0)


def kernel(x_ref, g_ref, wq_ref, wkT_ref, wvT_ref, wo_ref, w1T_ref, w3T_ref, w2_ref,
           out_ref, dx_ref, dwq_ref, dwkT_ref, dwvT_ref, dwo_ref, dw1T_ref, dw3T_ref, dw2_ref,
           xT_s, xnT_s, wqT_s, woT_s, w1_s, w3_s, w2T_s, wkv_s,
           k_s, v_s, kT_s, vT_s, qT_s, doT_s, delta_s, p0, p1, m0, m1, fin0, fin1,
           oT_s, dqT_s, hT_s, dhT_s, dk_acc, dv_acc, dxT_s,
           dwq_acc, dwo_acc, dw1_acc, dw3_acc, dw2_acc):
    i = pl.program_id(0)

    @pl.when(i == 0)
    def _prologue():
        wqT_s[...] = wq_ref[...].T
        woT_s[...] = wo_ref[...].T
        w1_s[...] = w1T_ref[...].T
        w3_s[...] = w3T_ref[...].T
        w2T_s[...] = w2_ref[...].T
        wkvT = jnp.concatenate([wkT_ref[...], wvT_ref[...]], axis=0)
        wkv_s[...] = wkvT.astype(f32).T.astype(bf16)
        for r in (dwq_acc, dwo_acc, dw1_acc, dw3_acc, dw2_acc, dk_acc, dv_acc):
            r[...] = jnp.zeros_like(r)

        def blk(b, c):
            r0 = pl.multiple_of(b * TQ, TQ)
            xT = x_ref[pl.ds(r0, TQ), :].astype(f32).T
            xT_s[b] = xT
            xn, _ = ln_stats(xT)
            xnb = xn.astype(bf16)
            xnT_s[b] = xnb
            kvT = dot(wkvT, xnb)
            kvTb = kvT.astype(bf16)
            kT_s[:, pl.ds(r0, TQ)] = as_u32(kvTb[0:DH])
            vT_s[:, pl.ds(r0, TQ)] = as_u32(kvTb[DH:2 * DH])
            kv = kvT.T.astype(bf16)
            r2 = pl.multiple_of(b * (TQ // 2), TQ // 2)
            k_s[pl.ds(r2, TQ // 2), :] = as_u32(kv[:, 0:DH])
            v_s[pl.ds(r2, TQ // 2), :] = as_u32(kv[:, DH:2 * DH])
            return c
        lax.fori_loop(0, NB, blk, 0)
        qT_s[0] = (dot(wqT_s[...], xnT_s[0]) * (SCALE * LOG2E)).astype(bf16)

    par = i % 2
    common = (k_s, v_s, kT_s, vT_s)
    tail = (oT_s, dqT_s, dk_acc, dv_acc)

    @pl.when(i == 0)
    def _():
        attention(True, False, *common, qT_s.at[0], qT_s.at[1], doT_s, delta_s,
                  p0, p1, m0, m1, fin0, fin1, *tail)

    @pl.when(jnp.logical_and(jnp.logical_and(i > 0, i < NB), par == 0))
    def _():
        attention(True, True, *common, qT_s.at[0], qT_s.at[1], doT_s, delta_s,
                  p0, p1, m0, m1, fin0, fin1, *tail)

    @pl.when(jnp.logical_and(i < NB, par == 1))
    def _():
        attention(True, True, *common, qT_s.at[1], qT_s.at[0], doT_s, delta_s,
                  p1, p0, m1, m0, fin1, fin0, *tail)

    @pl.when(i == NB)
    def _():
        attention(False, True, *common, qT_s.at[0], qT_s.at[1], doT_s, delta_s,
                  p0, p1, m0, m1, fin0, fin1, *tail)

    @pl.when(i > 0)
    def _post_bwd():
        j = i - 1
        dqb = (dqT_s[...] * SCALE).astype(bf16)
        dwq_acc[...] += dot(xnT_s[j], dqb, NT)
        dxn = dot(wq_ref[...], dqb)
        xn1, rstd1 = ln_stats(xT_s[j])
        dxT_s[j] = dhT_s[...] + ln_bwd(dxn, xn1, rstd1)

    @pl.when(i < NB)
    def _post_fwd():
        xT = xT_s[i]
        oT = oT_s[...]
        ob = oT.astype(bf16)
        hT = xT + dot(woT_s[...], ob)
        xn2, rstd2 = ln_stats(hT)
        xn2b = xn2.astype(bf16)
        g = dot(w1T_ref[...], xn2b)
        u = dot(w3T_ref[...], xn2b)
        sig = jax.nn.sigmoid(g)
        silu = g * sig
        hh = (silu * u).astype(bf16)
        outT = hT + dot(w2T_s[...], hh)
        out_ref[...] = outT.T.astype(bf16)

        doutT = g_ref[...].astype(f32).T
        doutb = doutT.astype(bf16)
        dhh = dot(w2_ref[...], doutb)
        dw2_acc[...] += dot(hh, doutb, NT)
        du = (dhh * silu).astype(bf16)
        dg = (dhh * u * (sig * (1.0 + g * (1.0 - sig)))).astype(bf16)
        dw1_acc[...] += dot(dg, xn2b, NT)
        dw3_acc[...] += dot(du, xn2b, NT)
        dxn2 = dot(w1_s[...], dg) + dot(w3_s[...], du)
        dhT = doutT + ln_bwd(dxn2, xn2, rstd2)
        dhT_s[...] = dhT
        dhb = dhT.astype(bf16)
        dwo_acc[...] += dot(ob, dhb, NT)
        doT = dot(wo_ref[...], dhb)
        doT_s[...] = doT
        delta = jnp.sum((doT * oT).reshape(H, DH, TQ), axis=1, keepdims=True)
        delta_s[...] = jnp.broadcast_to(delta, (H, 8, TQ))

    @pl.when(i < NB - 1)
    def _next_q():
        qT_s[1 - par] = (dot(wqT_s[...], xnT_s[i + 1]) * (SCALE * LOG2E)).astype(bf16)

    @pl.when(i == NB)
    def _epilogue():
        dkb = (dk_acc[...] * (1.0 / LOG2E)).astype(bf16)
        dvb = dv_acc[...].astype(bf16)
        kT_s[...] = as_u32(dkb)
        vT_s[...] = as_u32(dvb)

        def blk(b, c):
            r0 = pl.multiple_of(b * TQ, TQ)
            dkv = jnp.concatenate([as_bf16(kT_s[:, pl.ds(r0, TQ)]),
                                   as_bf16(vT_s[:, pl.ds(r0, TQ)])], axis=0)
            dxn_kv = dot(wkv_s[...], dkv)
            xn1, rstd1 = ln_stats(xT_s[b])
            dxT = dxT_s[b] + ln_bwd(dxn_kv, xn1, rstd1)
            dx_ref[pl.ds(r0, TQ), :] = dxT.T.astype(bf16)
            return c + dot(dkv, xnT_s[b], NT)
        dwkv = lax.fori_loop(0, NB, blk, jnp.zeros((2 * DH, D), f32))
        dwkT_ref[...] = dwkv[0:DH].astype(bf16)
        dwvT_ref[...] = dwkv[DH:2 * DH].astype(bf16)
        dwq_ref[...] = dwq_acc[...].astype(bf16)
        dwo_ref[...] = dwo_acc[...].astype(bf16)
        dw1T_ref[...] = dw1_acc[...].astype(bf16)
        dw3T_ref[...] = dw3_acc[...].astype(bf16)
        dw2_ref[...] = dw2_acc[...].astype(bf16)


def full(shape):
    return pl.BlockSpec(shape, lambda i: (0,) * len(shape))


@jax.jit
def pallas_sequential_preLN__grouped_kv_mqa__glu_gated_swiglu__prompt_kernel(
    A_x, A_wq, A_wk, A_wv, A_wo, B_x, B_w1, B_w3, B_w2, grad_out):
    x = A_x.reshape(S, D)
    g = grad_out.reshape(S, D)
    blkspec = pl.BlockSpec((TQ, D), lambda i: (jnp.minimum(i, NB - 1), 0))
    wshapes = [(D, D), (DH, D), (DH, D), (D, D), (F, D), (F, D), (F, D)]
    VM = pltpu.VMEM
    scratch = [
        VM((NB, D, TQ), f32), VM((NB, D, TQ), bf16),
        VM((D, D), bf16), VM((D, D), bf16), VM((D, F), bf16), VM((D, F), bf16), VM((D, F), bf16),
        VM((D, 2 * DH), bf16),
        VM((S // 2, DH), u32), VM((S // 2, DH), u32), VM((DH // 2, S), u32), VM((DH // 2, S), u32),
        VM((2, D, TQ), bf16), VM((D, TQ), f32), VM((H, 8, TQ), f32),
        VM((H, S, TQ), bf16), VM((H, S, TQ), bf16),
        VM((H, NC, 8, TQ), f32), VM((H, NC, 8, TQ), f32),
        VM((H, 2, 8, TQ), f32), VM((H, 2, 8, TQ), f32),
        VM((D, TQ), f32), VM((D, TQ), f32), VM((D, TQ), f32), VM((D, TQ), f32),
        VM((DH, S), f32), VM((DH, S), f32), VM((NB, D, TQ), f32),
        VM((D, D), f32), VM((D, D), f32), VM((F, D), f32), VM((F, D), f32), VM((F, D), f32),
    ]
    outs = pl.pallas_call(
        kernel,
        grid=(NB + 1,),
        in_specs=[full((S, D)), blkspec] + [full(s) for s in wshapes],
        out_specs=[blkspec, full((S, D))] + [full(s) for s in wshapes],
        out_shape=[jax.ShapeDtypeStruct((S, D), bf16), jax.ShapeDtypeStruct((S, D), bf16)]
        + [jax.ShapeDtypeStruct(s, bf16) for s in wshapes],
        scratch_shapes=scratch,
        compiler_params=pltpu.CompilerParams(
            dimension_semantics=("arbitrary",), vmem_limit_bytes=120 * 2**20),
        name="fused_block",
    )(x, g, A_wq, A_wk.T, A_wv.T, A_wo, B_w1.T, B_w3.T, B_w2)
    out, dx, dwq, dwkT, dwvT, dwo, dw1T, dw3T, dw2 = outs
    return (out.reshape(1, S, D), dx.reshape(1, S, D), dwq, dwkT.T, dwvT.T, dwo,
            dw1T.T, dw3T.T, dw2)
```

```python
import jax
import jax.numpy as jnp
from jax import lax
import jax.experimental.pallas as pl
import jax.experimental.pallas.tpu as pltpu

S, D, H, DH, F = 2048, 512, 32, 16, 1376
TQ = 128
NB = S // TQ
OC = 128
NC = S // OC
EPS = 1e-5
LOG2E = 1.4426950408889634
SCALE = DH ** -0.5
bf16 = jnp.bfloat16
f32 = jnp.float32
u32 = jnp.uint32
NN = (((1,), (0,)), ((), ()))
NT = (((1,), (1,)), ((), ()))

import os
def _cfg(name, default):
    v = os.environ.get(name, default).split(",")
    return tuple(int(t) for t in v[:6]) + (v[6],)
CFG_M = _cfg("KM", "8,64,64,6,5,4,SDVKPQ")
CFG_F = _cfg("KF", "8,32,64,8,5,4,SDVKPQ")
CFG_B = _cfg("KB", "8,64,64,6,6,4,SDVKPQ")
PAD = [int(v) for v in os.environ.get("KPAD", "8,8,8").split(",")]


def dot(a, b, dn=NN):
    return lax.dot_general(a, b, dn, preferred_element_type=f32)


def as_u32(x):
    return pltpu.bitcast(x, u32)


def as_bf16(x):
    return pltpu.bitcast(x, bf16)


def ln_stats(xT, with_mu=False):
    mu = jnp.mean(xT, axis=0, keepdims=True)
    xc = xT - mu
    var = jnp.mean(xc * xc, axis=0, keepdims=True)
    rstd = 1.0 / jnp.sqrt(var + EPS)
    return (xc * rstd, rstd, mu) if with_mu else (xc * rstd, rstd)


def ln_bwd(dxn, xn, rstd):
    m1 = jnp.mean(dxn, axis=0, keepdims=True)
    m2 = jnp.mean(dxn * xn, axis=0, keepdims=True)
    return rstd * (dxn - m1 - xn * m2)


def ln_bwd_cached(d, x, mu, rstd):
    n = d.shape[0]
    m1 = jnp.sum(d, axis=0, keepdims=True) * (1.0 / n)
    m2 = rstd * (jnp.sum(d * x, axis=0, keepdims=True) * (1.0 / n) - mu * m1)
    b = -(rstd * rstd) * m2
    return rstd * d + (b * x + (-rstd * m1 - b * mu))


def hs(h):
    return pl.ds(pl.multiple_of(h * DH, DH), DH)


def attention(cfg, fwd, bwd, k_s, v_s, kT_s, vT_s, qF, qB, doT_s, delta_s, pF, pB, mF, mB,
              finF, finB, oT_s, dqT_s, dk_acc, dv_acc):
    U, LRS, LRD, SKEW_P, SKEW_K, SKEW_V, ORDER = cfg
    carry_p = fwd and not bwd
    def lhs(ref, r0, n):
        return as_bf16(ref[r0 // 2:(r0 + n) // 2, :])

    def tT(ref, c):
        return as_bf16(ref[:, c * OC:(c + 1) * OC])

    def cr(c):
        return slice(c * OC, (c + 1) * OC)

    def long_dot(ref, c, w, lr):
        parts = [dot(lhs(ref, c * OC + j * lr, lr), w) for j in range(OC // lr)]
        return parts[0] if len(parts) == 1 else jnp.concatenate(parts, axis=0)

    def finish_head(h, o, m, l):
        linv = 1.0 / jnp.sum(l, axis=0, keepdims=True)
        oT_s[hs(h + 1), :] = o * linv
        finF[h + 1, 0] = jnp.broadcast_to(m, (8, TQ))
        finF[h + 1, 1] = jnp.broadcast_to(linv, (8, TQ))

    def pv(h, c, o, al):
        return o * al + dot(tT(vT_s, c), pF[h + 1, cr(c), :])

    def block(i, carry):
        hprev = i * U - 1
        prev = dict(o=carry[0]) if carry_p else None
        hh = [i * U + u for u in range(U)]
        st = [dict(alpha={}, ds={}, w={}) for _ in hh]
        for u, h in enumerate(hh):
            s_ = st[u]
            if fwd:
                s_["q"] = qF[hs(h), :]
                s_["m"] = jnp.full((1, TQ), -1e30, f32)
                s_["l"] = jnp.zeros((8, TQ), f32)
                s_["o"] = jnp.zeros((DH, TQ), f32)
            if bwd:
                s_["qb"] = qB[hs(h), :]
                s_["do"] = doT_s[hs(h), :]
                s_["delta"] = delta_s[h]
                s_["mfin"] = finB[h + 1, 0]
                s_["linv"] = finB[h + 1, 1]
                s_["dq"] = jnp.zeros((DH, TQ), f32)
        T = U * NC

        def S_(t):
            u, c = divmod(t, NC)
            s_ = st[u]
            s = long_dot(k_s, c, s_["q"], LRS)
            mn = jnp.maximum(s_["m"], jnp.max(s, axis=0, keepdims=True))
            p = jnp.exp2(s - mn)
            al = jnp.exp2(s_["m"] - mn)
            s_["l"] = s_["l"] * al + p.reshape(OC // 8, 8, TQ).sum(axis=0)
            pF[hh[u] + 1, cr(c), :] = p.astype(bf16)
            mF[hh[u], c] = jnp.broadcast_to(mn, (8, TQ))
            s_["m"] = mn
            s_["alpha"][c] = al

        def P_(t):
            u, c = divmod(t, NC)
            s_ = st[u]
            s_["o"] = pv(hh[u], c, s_["o"], s_["alpha"].pop(c))
            if c == NC - 1:
                finish_head(hh[u], s_["o"], s_["m"], s_["l"])

        def Pprev_(n):
            prev["o"] = pv(hprev, NC - SKEW_P + n, prev["o"], carry[3 + n])
            if n == SKEW_P - 1:
                finish_head(hprev, prev["o"], carry[1], carry[2])

        def W_(u, c):
            s_ = st[u]
            if c not in s_["w"]:
                corr = jnp.exp2(mB[hh[u], c] - s_["mfin"]) * s_["linv"]
                w = (s_["do"].reshape(2, 8, TQ) * corr).reshape(DH, TQ).astype(bf16)
                s_["w"][c] = (w, (s_["delta"] * corr)[0:1, :])
            return s_["w"][c]

        def D_(t):
            u, c = divmod(t, NC)
            w, dl = W_(u, c)
            dp = long_dot(v_s, c, w, LRD)
            st[u]["ds"][c] = (pB[hh[u] + 1, cr(c), :].astype(f32) * (dp - dl)).astype(bf16)

        def V_(t):
            u, c = divmod(t, NC)
            dv_acc[:, cr(c)] += dot(W_(u, c)[0], pB[hh[u] + 1, cr(c), :], NT)

        def K_(t):
            u, c = divmod(t, NC)
            dk_acc[:, cr(c)] += dot(st[u]["qb"], st[u]["ds"][c], NT)

        def Q_(t):
            u, c = divmod(t, NC)
            s_ = st[u]
            s_["dq"] = s_["dq"] + dot(tT(kT_s, c), s_["ds"].pop(c))
            if c == NC - 1:
                dqT_s[hs(hh[u]), :] = s_["dq"]

        for t in range(T + (0 if carry_p else max(SKEW_P, SKEW_K, SKEW_V))):
            for op in ORDER:
                if op == "S" and fwd and t < T:
                    S_(t)
                if op == "P" and fwd:
                    if carry_p and t < SKEW_P:
                        Pprev_(t)
                    elif 0 <= t - SKEW_P < T:
                        P_(t - SKEW_P)
                if op == "D" and bwd and t < T:
                    D_(t)
                if op == "V" and bwd and 0 <= t - SKEW_V < T:
                    V_(t - SKEW_V)
                if op == "K" and bwd and 0 <= t - SKEW_K < T:
                    K_(t - SKEW_K)
                if op == "Q" and bwd and 0 <= t - SKEW_K < T:
                    Q_(t - SKEW_K)
        if not carry_p:
            return carry
        last = st[U - 1]
        return (last["o"], last["m"], last["l"]) + tuple(last["alpha"][c] for c in range(NC - SKEW_P, NC))

    if carry_p:
        init = (jnp.zeros((DH, TQ), f32), jnp.zeros((1, TQ), f32), jnp.ones((8, TQ), f32)) \
            + tuple(jnp.zeros((1, TQ), f32) for _ in range(SKEW_P))
        carry = lax.fori_loop(0, H // U, block, init)
        o = carry[0]
        for n in range(SKEW_P):
            o = pv(H - 1, NC - SKEW_P + n, o, carry[3 + n])
        finish_head(H - 1, o, carry[1], carry[2])
    else:
        lax.fori_loop(0, H // U, block, 0)


def kernel(x_hbm, g_ref, wq_hbm, wkT_hbm, wvT_hbm, wo_hbm, w1T_hbm, w3T_hbm, w2_hbm,
           out_ref, dx_hbm, dwq_hbm, dwkT_hbm, dwvT_hbm, dwo_hbm, dw1T_hbm, dw3T_hbm, dw2_hbm,
           x_v, wq_v, wkT_v, wvT_v, wo_v, w1T_v, w3T_v, w2_v, dx_v, dwq_v, dwkv_v,
           xT_s, xnT_s, st1_s, kvf_s, dkv_s, wqT_s, woT_s, w1_s, w3_s, w2T_s, wkv_s,
           k_s, v_s, kT_s, vT_s, qT_s, doT_s, delta_s, pad0, p0, pad1, p1, pad2, m0, m1, fin0, fin1,
           oT_s, dqT_s, dhT_s, dk_acc, dv_acc, dxT_s,
           dwq_acc, dwo_acc, dw1_acc, dw3_acc, dw2_acc, sem):
    i = pl.program_id(0)
    XC = 4
    XR = S // XC

    def rows(c):
        return pl.ds(pl.multiple_of(c * XR, XR), XR)

    def x_copy(c):
        return pltpu.make_async_copy(x_hbm.at[rows(c)], x_v.at[rows(c)], sem.at[c])

    def dx_copy(c):
        return pltpu.make_async_copy(dx_v.at[rows(c)], dx_hbm.at[rows(c)], sem.at[c])

    first = [pltpu.make_async_copy(a, b, sem.at[XC + n]) for n, (a, b) in enumerate(
        [(wkT_hbm, wkT_v), (wvT_hbm, wvT_v), (wq_hbm, wq_v)])]
    late = [pltpu.make_async_copy(a, b, sem.at[XC + 3 + n]) for n, (a, b) in enumerate(
        [(wo_hbm, wo_v), (w1T_hbm, w1T_v), (w3T_hbm, w3T_v), (w2_hbm, w2_v)])]
    grads = [pltpu.make_async_copy(a, b, sem.at[XC + 3 + n]) for n, (a, b) in enumerate(
        [(wo_v, dwo_hbm), (w1T_v, dw1T_hbm), (w3T_v, dw3T_hbm), (w2_v, dw2_hbm)])]
    dwq_copy = pltpu.make_async_copy(dwq_v, dwq_hbm, sem.at[XC])
    dwk_copy = pltpu.make_async_copy(dwkv_v.at[pl.ds(0, DH)], dwkT_hbm, sem.at[XC + 1])
    dwv_copy = pltpu.make_async_copy(dwkv_v.at[pl.ds(DH, DH)], dwvT_hbm, sem.at[XC + 2])

    @pl.when(i == 0)
    def _prologue():
        for c in first:
            c.start()
        for c in range(XC):
            x_copy(c).start()
        for c in late:
            c.start()
        for r in (dk_acc, dv_acc, dqT_s, dhT_s):
            r[...] = jnp.zeros_like(r)
        for c in first:
            c.wait()
        wqT_s[...] = wq_v[...].T
        wkvT = jnp.concatenate([wkT_v[...], wvT_v[...]], axis=0)
        wkv_s[...] = wkvT.astype(f32).T.astype(bf16)
        def chunk(c, carry):
            x_copy(c).wait()
            for bb in range(NB // XC):
                b = c * (NB // XC) + bb
                r0 = pl.multiple_of(b * TQ, TQ)
                xT = x_v[pl.ds(r0, TQ), :].astype(f32).T
                xT_s[b] = xT
                xn, rstd1, mu1 = ln_stats(xT, True)
                st1_s[b, 0] = jnp.broadcast_to(mu1, (8, TQ))
                st1_s[b, 1] = jnp.broadcast_to(rstd1, (8, TQ))
                xnT_s[b] = xn.astype(bf16)
            return carry
        lax.fori_loop(0, XC, chunk, 0)
        for b in range(NB):
            cols = slice(b * TQ, (b + 1) * TQ)
            kvT = dot(wkvT, xnT_s[b])
            kvf_s[:, cols] = kvT
            kT_s[:, cols] = as_u32(kvT[0:DH].astype(bf16))
            vT_s[:, cols] = as_u32(kvT[DH:2 * DH].astype(bf16))
            kv = kvT.T
            rows2 = slice(b * (TQ // 2), (b + 1) * (TQ // 2))
            k_s[rows2, :] = as_u32(kv[:, 0:DH].astype(bf16))
            v_s[rows2, :] = as_u32(kv[:, DH:2 * DH].astype(bf16))
        qT_s[0] = (dot(wqT_s[...], xnT_s[0]) * (SCALE * LOG2E)).astype(bf16)

    par = i % 2
    common = (k_s, v_s, kT_s, vT_s)
    tail = (oT_s, dqT_s, dk_acc, dv_acc)

    @pl.when(i == 0)
    def _():
        attention(CFG_F, True, False, *common, qT_s.at[0], qT_s.at[1], doT_s, delta_s,
                  p0, p1, m0, m1, fin0, fin1, *tail)

    @pl.when(i == 0)
    def _late_weights():
        for c in late:
            c.wait()
        woT_s[...] = wo_v[...].T
        w1_s[...] = w1T_v[...].T
        w3_s[...] = w3T_v[...].T
        w2T_s[...] = w2_v[...].T

    @pl.when(i == NB)
    def _early_grads():
        wo_v[...] = dwo_acc[...].astype(bf16)
        w1T_v[...] = dw1_acc[...].astype(bf16)
        w3T_v[...] = dw3_acc[...].astype(bf16)
        w2_v[...] = dw2_acc[...].astype(bf16)
        for c in grads:
            c.start()

    @pl.when(jnp.logical_and(jnp.logical_and(i > 0, i < NB), par == 0))
    def _():
        attention(CFG_M, True, True, *common, qT_s.at[0], qT_s.at[1], doT_s, delta_s,
                  p0, p1, m0, m1, fin0, fin1, *tail)

    @pl.when(jnp.logical_and(i < NB, par == 1))
    def _():
        attention(CFG_M, True, True, *common, qT_s.at[1], qT_s.at[0], doT_s, delta_s,
                  p1, p0, m1, m0, fin1, fin0, *tail)

    @pl.when(i == NB)
    def _():
        attention(CFG_B, False, True, *common, qT_s.at[0], qT_s.at[1], doT_s, delta_s,
                  p0, p1, m0, m1, fin0, fin1, *tail)

    def accumulate(ref, val):
        ref[...] = jnp.where(i > 0, ref[...], 0.0) + val

    def post_bwd(j):
        dqb = (dqT_s[...] * SCALE).astype(bf16)
        dxn = dot(wq_v[...], dqb)
        accumulate(dwq_acc, dot(xnT_s[j], dqb, NT))
        dxT_s[j] = dhT_s[...] + ln_bwd_cached(dxn, xT_s[j], st1_s[j, 0][0:1], st1_s[j, 1][0:1])

    @pl.when(i < NB)
    def _dense():
        doutT = g_ref[...].astype(f32).T
        doutb = doutT.astype(bf16)
        xT = xT_s[i]
        oT = oT_s[DH:DH + D, :]
        ob = oT.astype(bf16)
        hT = xT + dot(woT_s[...], ob)
        dhh = dot(w2_v[...], doutb)
        post_bwd(jnp.maximum(i - 1, 0))
        xn2, rstd2 = ln_stats(hT)
        xn2b = xn2.astype(bf16)
        g = dot(w1T_v[...], xn2b)
        u = dot(w3T_v[...], xn2b)
        sig = jax.nn.sigmoid(g)
        silu = g * sig
        hh = (silu * u).astype(bf16)
        du = (dhh * silu).astype(bf16)
        dg = (dhh * u * (sig * (1.0 + g * (1.0 - sig)))).astype(bf16)
        outT = hT + dot(w2T_s[...], hh)
        out_ref[...] = outT.T.astype(bf16)
        dxn2 = dot(w1_s[...], dg) + dot(w3_s[...], du)
        accumulate(dw2_acc, dot(hh, doutb, NT))
        accumulate(dw1_acc, dot(dg, xn2b, NT))
        accumulate(dw3_acc, dot(du, xn2b, NT))
        dhT = doutT + ln_bwd(dxn2, xn2, rstd2)
        dhT_s[...] = dhT
        dhb = dhT.astype(bf16)
        doT = dot(wo_v[...], dhb)
        accumulate(dwo_acc, dot(ob, dhb, NT))
        qT_s[1 - par] = (dot(wqT_s[...], xnT_s[jnp.minimum(i + 1, NB - 1)])
                         * (SCALE * LOG2E)).astype(bf16)
        doT_s[...] = doT
        delta = jnp.sum((doT * oT).reshape(H, DH, TQ), axis=1, keepdims=True)
        delta_s[...] = jnp.broadcast_to(delta, (H, 8, TQ))

    @pl.when(i == NB)
    def _epilogue():
        post_bwd(NB - 1)
        dwq_v[...] = dwq_acc[...].astype(bf16)
        dwq_copy.start()
        for b in range(NB):
            cols = slice(b * TQ, (b + 1) * TQ)
            dkv_s[b, 0:DH] = (dk_acc[:, cols] * (1.0 / LOG2E)).astype(bf16)
            dkv_s[b, DH:2 * DH] = dv_acc[:, cols].astype(bf16)
        wkvT = jnp.concatenate([wkT_v[...], wvT_v[...]], axis=0).astype(f32)
        wbar = jnp.sum(wkvT, axis=1, keepdims=True) * (1.0 / D)

        def chunk(c, dwkv):
            for bb in range(NB // XC):
                b = c * (NB // XC) + bb
                r0 = pl.multiple_of(b * TQ, TQ)
                dkv = dkv_s[b]
                d = dot(wkv_s[...], dkv)
                dkf = dkv.astype(f32)
                m1 = jnp.sum(wbar * dkf, axis=0, keepdims=True)
                m2 = jnp.sum(kvf_s[:, pl.ds(r0, TQ)] * dkf, axis=0, keepdims=True) * (1.0 / D)
                mu, rstd = st1_s[b, 0][0:1], st1_s[b, 1][0:1]
                bx = -(rstd * rstd) * m2
                dxT = dxT_s[b] + rstd * d + (bx * xT_s[b] + (-rstd * m1 - bx * mu))
                dx_v[pl.ds(r0, TQ), :] = dxT.T.astype(bf16)
                dwkv = dwkv + dot(dkv, xnT_s[b], NT)
            dx_copy(c).start()
            return dwkv
        dwkv = lax.fori_loop(0, XC, chunk, jnp.zeros((2 * DH, D), f32))
        dwkv_v[...] = dwkv.astype(bf16)
        dwk_copy.start()
        dwv_copy.start()
        for c in grads:
            c.wait()
        dwq_copy.wait()
        dwk_copy.wait()
        dwv_copy.wait()
        for c in range(XC):
            dx_copy(c).wait()


@jax.jit
def pallas_sequential_preLN__grouped_kv_mqa__glu_gated_swiglu__prompt_kernel(
    A_x, A_wq, A_wk, A_wv, A_wo, B_x, B_w1, B_w3, B_w2, grad_out):
    x = A_x.reshape(S, D)
    g = grad_out.reshape(S, D)
    blkspec = pl.BlockSpec((TQ, D), lambda i: (jnp.minimum(i, NB - 1), 0))
    anyspec = pl.BlockSpec(memory_space=pl.ANY)
    wshapes = [(D, D), (DH, D), (DH, D), (D, D), (F, D), (F, D), (F, D)]
    VM = pltpu.VMEM
    scratch = [
        VM((S, D), bf16), VM((D, D), bf16), VM((DH, D), bf16), VM((DH, D), bf16), VM((D, D), bf16),
        VM((F, D), bf16), VM((F, D), bf16), VM((F, D), bf16),
        VM((S, D), bf16), VM((D, D), bf16), VM((2 * DH, D), bf16),
        VM((NB, D, TQ), f32), VM((NB, D, TQ), bf16), VM((NB, 2, 8, TQ), f32), VM((2 * DH, S), f32), VM((NB, 2 * DH, TQ), bf16),
        VM((D, D), bf16), VM((D, D), bf16), VM((D, F), bf16), VM((D, F), bf16), VM((D, F), bf16),
        VM((D, 2 * DH), bf16),
        VM((S // 2, DH), u32), VM((S // 2, DH), u32), VM((DH // 2, S), u32), VM((DH // 2, S), u32),
        VM((2, D, TQ), bf16), VM((D, TQ), f32), VM((H, 8, TQ), f32),
        VM((PAD[0], TQ), f32), VM((H + 1, S, TQ), bf16), VM((PAD[1], TQ), f32), VM((H + 1, S, TQ), bf16), VM((PAD[2], TQ), f32),
        VM((H, NC, 8, TQ), f32), VM((H, NC, 8, TQ), f32),
        VM((H + 1, 2, 8, TQ), f32), VM((H + 1, 2, 8, TQ), f32),
        VM((D + DH, TQ), f32), VM((D, TQ), f32), VM((D, TQ), f32),
        VM((DH, S), f32), VM((DH, S), f32), VM((NB, D, TQ), f32),
        VM((D, D), f32), VM((D, D), f32), VM((F, D), f32), VM((F, D), f32), VM((F, D), f32),
        pltpu.SemaphoreType.DMA((12,)),
    ]
    outs = pl.pallas_call(
        kernel,
        grid=(NB + 1,),
        in_specs=[anyspec, blkspec] + [anyspec] * len(wshapes),
        out_specs=[blkspec, anyspec] + [anyspec] * len(wshapes),
        out_shape=[jax.ShapeDtypeStruct((S, D), bf16), jax.ShapeDtypeStruct((S, D), bf16)]
        + [jax.ShapeDtypeStruct(s, bf16) for s in wshapes],
        scratch_shapes=scratch,
        compiler_params=pltpu.CompilerParams(
            dimension_semantics=("arbitrary",), vmem_limit_bytes=120 * 2**20),
        name="fused_block",
    )(x, g, A_wq, A_wk.T, A_wv.T, A_wo, B_w1.T, B_w3.T, B_w2)
    out, dx, dwq, dwkT, dwvT, dwo, dw1T, dw3T, dw2 = outs
    return (out.reshape(1, S, D), dx.reshape(1, S, D), dwq, dwkT.T, dwvT.T, dwo,
            dw1T.T, dw3T.T, dw2)
```

```python
import jax
import jax.numpy as jnp
from jax import lax
import jax.experimental.pallas as pl
import jax.experimental.pallas.tpu as pltpu

S, D, H, DH, F = 2048, 512, 32, 16, 1376
TQ = 128
NB = S // TQ
OC = 128
NC = S // OC
EPS = 1e-5
LOG2E = 1.4426950408889634
SCALE = DH ** -0.5
bf16 = jnp.bfloat16
f32 = jnp.float32
u32 = jnp.uint32
NN = (((1,), (0,)), ((), ()))
NT = (((1,), (1,)), ((), ()))

CFG_M = (8, 64, 64, 6, 5, 0, "SDVKPQ")
CFG_F = (8, 32, 64, 8, 5, 4, "SDVKPQ")
CFG_B = (8, 64, 64, 6, 6, 4, "SDVKPQ")
FP = 352
FPAD = 4 * FP
FPIECES = ((0, 96), (96, 96), (192, 80), (272, 80))


def dot(a, b, dn=NN):
    return lax.dot_general(a, b, dn, preferred_element_type=f32)


def as_u32(x):
    return pltpu.bitcast(x, u32)


def as_bf16(x):
    return pltpu.bitcast(x, bf16)


def ln_stats(xT, with_mu=False):
    mu = jnp.mean(xT, axis=0, keepdims=True)
    xc = xT - mu
    var = jnp.mean(xc * xc, axis=0, keepdims=True)
    rstd = 1.0 / jnp.sqrt(var + EPS)
    return (xc * rstd, rstd, mu) if with_mu else (xc * rstd, rstd)


def ln_bwd(dxn, xn, rstd):
    m1 = jnp.mean(dxn, axis=0, keepdims=True)
    m2 = jnp.mean(dxn * xn, axis=0, keepdims=True)
    return rstd * (dxn - m1 - xn * m2)


def ln_bwd_cached(d, x, mu, rstd):
    n = d.shape[0]
    m1 = jnp.sum(d, axis=0, keepdims=True) * (1.0 / n)
    m2 = rstd * (jnp.sum(d * x, axis=0, keepdims=True) * (1.0 / n) - mu * m1)
    b = -(rstd * rstd) * m2
    return rstd * d + (b * x + (-rstd * m1 - b * mu))


def hs(h):
    return pl.ds(pl.multiple_of(h * DH, DH), DH)


def attention(cfg, fwd, bwd, k_s, v_s, kT_s, vT_s, qF, qB, doT_s, delta_s, pF, pB, mF, mB,
              finF, finB, oT_s, dqT_s, dk_acc, dv_acc, filler=None):
    U, LRS, LRD, SKEW_P, SKEW_K, SKEW_V, ORDER = cfg
    carry_p = fwd and not bwd
    def lhs(ref, r0, n):
        return as_bf16(ref[r0 // 2:(r0 + n) // 2, :])

    def tT(ref, c):
        return as_bf16(ref[:, c * OC:(c + 1) * OC])

    def cr(c):
        return slice(c * OC, (c + 1) * OC)

    def long_dot(ref, c, w, lr):
        parts = [dot(lhs(ref, c * OC + j * lr, lr), w) for j in range(OC // lr)]
        return parts[0] if len(parts) == 1 else jnp.concatenate(parts, axis=0)

    def finish_head(h, o, m, l):
        linv = 1.0 / jnp.sum(l, axis=0, keepdims=True)
        oT_s[hs(h + 1), :] = o * linv
        finF[h + 1, 0] = jnp.broadcast_to(m, (8, TQ))
        finF[h + 1, 1] = jnp.broadcast_to(linv, (8, TQ))

    def pv(h, c, o, al):
        return o * al + dot(tT(vT_s, c), pF[h + 1, cr(c), :])

    def block(i, carry):
        hprev = i * U - 1
        prev = dict(o=carry[0]) if carry_p else None
        hh = [i * U + u for u in range(U)]
        st = [dict(alpha={}, ds={}, w={}) for _ in hh]
        for u, h in enumerate(hh):
            s_ = st[u]
            if fwd:
                s_["q"] = qF[hs(h), :]
                s_["m"] = jnp.full((1, TQ), -1e30, f32)
                s_["l"] = jnp.zeros((8, TQ), f32)
                s_["o"] = jnp.zeros((DH, TQ), f32)
            if bwd:
                s_["qb"] = qB[hs(h), :]
                s_["do"] = doT_s[hs(h), :]
                s_["delta"] = delta_s[h]
                s_["mfin"] = finB[h + 1, 0]
                s_["linv"] = finB[h + 1, 1]
                s_["dq"] = jnp.zeros((DH, TQ), f32)
        T = U * NC

        def S_(t):
            u, c = divmod(t, NC)
            s_ = st[u]
            s = long_dot(k_s, c, s_["q"], LRS)
            mn = jnp.maximum(s_["m"], jnp.max(s, axis=0, keepdims=True))
            p = jnp.exp2(s - mn)
            al = jnp.exp2(s_["m"] - mn)
            s_["l"] = s_["l"] * al + p.reshape(OC // 8, 8, TQ).sum(axis=0)
            pF[hh[u] + 1, cr(c), :] = p.astype(bf16)
            mF[hh[u], c] = jnp.broadcast_to(mn, (8, TQ))
            s_["m"] = mn
            s_["alpha"][c] = al

        def P_(t):
            u, c = divmod(t, NC)
            s_ = st[u]
            s_["o"] = pv(hh[u], c, s_["o"], s_["alpha"].pop(c))
            if c == NC - 1:
                finish_head(hh[u], s_["o"], s_["m"], s_["l"])

        def Pprev_(n):
            prev["o"] = pv(hprev, NC - SKEW_P + n, prev["o"], carry[3 + n])
            if n == SKEW_P - 1:
                finish_head(hprev, prev["o"], carry[1], carry[2])

        def W_(u, c):
            s_ = st[u]
            if c not in s_["w"]:
                corr = jnp.exp2(mB[hh[u], c] - s_["mfin"]) * s_["linv"]
                w = (s_["do"].reshape(2, 8, TQ) * corr).reshape(DH, TQ).astype(bf16)
                s_["w"][c] = (w, (s_["delta"] * corr)[0:1, :])
            return s_["w"][c]

        def D_(t):
            u, c = divmod(t, NC)
            w, dl = W_(u, c)
            dp = long_dot(v_s, c, w, LRD)
            st[u]["ds"][c] = (pB[hh[u] + 1, cr(c), :].astype(f32) * (dp - dl)).astype(bf16)

        def V_(t):
            u, c = divmod(t, NC)
            dv_acc[:, cr(c)] += dot(W_(u, c)[0], pB[hh[u] + 1, cr(c), :], NT)

        def K_(t):
            u, c = divmod(t, NC)
            dk_acc[:, cr(c)] += dot(st[u]["qb"], st[u]["ds"][c], NT)

        def Q_(t):
            u, c = divmod(t, NC)
            s_ = st[u]
            s_["dq"] = s_["dq"] + dot(tT(kT_s, c), s_["ds"].pop(c))
            if c == NC - 1:
                dqT_s[hs(hh[u]), :] = s_["dq"]

        for t in range(T + (0 if carry_p else max(SKEW_P, SKEW_K, SKEW_V))):
            if filler is not None and 0 <= t - T < len(FPIECES):
                filler(i, *FPIECES[t - T])
            for op in ORDER:
                if op == "S" and fwd and t < T:
                    S_(t)
                if op == "P" and fwd:
                    if carry_p and t < SKEW_P:
                        Pprev_(t)
                    elif 0 <= t - SKEW_P < T:
                        P_(t - SKEW_P)
                if op == "D" and bwd and t < T:
                    D_(t)
                if op == "V" and bwd and 0 <= t - SKEW_V < T:
                    V_(t - SKEW_V)
                if op == "K" and bwd and 0 <= t - SKEW_K < T:
                    K_(t - SKEW_K)
                if op == "Q" and bwd and 0 <= t - SKEW_K < T:
                    Q_(t - SKEW_K)
        if not carry_p:
            return carry
        last = st[U - 1]
        return (last["o"], last["m"], last["l"]) + tuple(last["alpha"][c] for c in range(NC - SKEW_P, NC))

    if carry_p:
        init = (jnp.zeros((DH, TQ), f32), jnp.zeros((1, TQ), f32), jnp.ones((8, TQ), f32)) \
            + tuple(jnp.zeros((1, TQ), f32) for _ in range(SKEW_P))
        carry = lax.fori_loop(0, H // U, block, init)
        o = carry[0]
        for n in range(SKEW_P):
            o = pv(H - 1, NC - SKEW_P + n, o, carry[3 + n])
        finish_head(H - 1, o, carry[1], carry[2])
    else:
        lax.fori_loop(0, H // U, block, 0)


def kernel(x_hbm, g_hbm, wq_hbm, wkT_hbm, wvT_hbm, wo_hbm, w1T_hbm, w3T_hbm, w2_hbm,
           out_hbm, dx_hbm, dwq_hbm, dwkT_hbm, dwvT_hbm, dwo_hbm, dw1T_hbm, dw3T_hbm, dw2_hbm,
           x_v, g_v, out_v, wq_v, wkT_v, wvT_v, wo_v, w1T_v, w3T_v, w2_v, dx_v, dwq_v, dwkv_v,
           xT_s, xnT_s, st1_s, kvf_s, dkv_s, wqT_s, woT_s, w1_s, w3_s, w2T_s, wkv_s,
           k_s, v_s, kT_s, vT_s, qT_s, doT_s, delta_s, p0, p1, m0, m1, fin0, fin1,
           oT_s, dqT_s, dhT_s, dhh_s, doutT_s, doutb_s, dk_acc, dv_acc, dxT_s,
           dwq_acc, dwo_acc, dw1_acc, dw3_acc, dw2_acc, sem):
    i = pl.program_id(0)
    XC = 4
    XR = S // XC

    def rows(c):
        return pl.ds(pl.multiple_of(c * XR, XR), XR)

    def x_copy(c):
        return pltpu.make_async_copy(x_hbm.at[rows(c)], x_v.at[rows(c)], sem.at[c])

    def dx_copy(c):
        return pltpu.make_async_copy(dx_v.at[rows(c)], dx_hbm.at[rows(c)], sem.at[c])

    def blk_rows(b):
        return pl.ds(pl.multiple_of(b * TQ, TQ), TQ)

    def out_copy(b):
        return pltpu.make_async_copy(out_v.at[b % 2], out_hbm.at[blk_rows(b)], sem.at[XC + 8 + b % 2])

    g_copy = pltpu.make_async_copy(g_hbm, g_v, sem.at[XC + 7])
    first = [pltpu.make_async_copy(a, b, sem.at[XC + n]) for n, (a, b) in enumerate(
        [(wkT_hbm, wkT_v), (wvT_hbm, wvT_v), (wq_hbm, wq_v)])]
    late = [pltpu.make_async_copy(a, b, sem.at[XC + 3 + n]) for n, (a, b) in enumerate(
        [(wo_hbm, wo_v), (w1T_hbm, w1T_v), (w3T_hbm, w3T_v), (w2_hbm, w2_v.at[pl.ds(0, F)])])]
    grads = [pltpu.make_async_copy(a, b, sem.at[XC + 3 + n]) for n, (a, b) in enumerate(
        [(wo_v, dwo_hbm), (w1T_v, dw1T_hbm), (w3T_v, dw3T_hbm), (w2_v.at[pl.ds(0, F)], dw2_hbm)])]
    dwq_copy = pltpu.make_async_copy(dwq_v, dwq_hbm, sem.at[XC])
    dwk_copy = pltpu.make_async_copy(dwkv_v.at[pl.ds(0, DH)], dwkT_hbm, sem.at[XC + 1])
    dwv_copy = pltpu.make_async_copy(dwkv_v.at[pl.ds(DH, DH)], dwvT_hbm, sem.at[XC + 2])

    @pl.when(i == 0)
    def _prologue():
        for c in range(XC):
            x_copy(c).start()
        for c in first:
            c.start()
        g_copy.start()
        for c in late:
            c.start()
        w2_v[F:FPAD, :] = jnp.zeros((FPAD - F, D), bf16)
        for r in (dk_acc, dv_acc, dqT_s, dhT_s):
            r[...] = jnp.zeros_like(r)
        p0[0] = jnp.zeros((S, TQ), bf16)

        def chunk(c, carry):
            x_copy(c).wait()
            for bb in range(NB // XC):
                b = c * (NB // XC) + bb
                r0 = pl.multiple_of(b * TQ, TQ)
                xT = x_v[pl.ds(r0, TQ), :].astype(f32).T
                xT_s[b] = xT
                xn, rstd1, mu1 = ln_stats(xT, True)
                st1_s[b, 0] = jnp.broadcast_to(mu1, (8, TQ))
                st1_s[b, 1] = jnp.broadcast_to(rstd1, (8, TQ))
                xnT_s[b] = xn.astype(bf16)
            return carry
        lax.fori_loop(0, XC, chunk, 0)
        for c in first:
            c.wait()
        wqT_s[...] = wq_v[...].T
        wkvT = jnp.concatenate([wkT_v[...], wvT_v[...]], axis=0)
        wkv_s[...] = wkvT.astype(f32).T.astype(bf16)
        for b in range(NB):
            cols = slice(b * TQ, (b + 1) * TQ)
            kvT = dot(wkvT, xnT_s[b])
            kvf_s[:, cols] = kvT
            kT_s[:, cols] = as_u32(kvT[0:DH].astype(bf16))
            vT_s[:, cols] = as_u32(kvT[DH:2 * DH].astype(bf16))
            kv = kvT.T
            rows2 = slice(b * (TQ // 2), (b + 1) * (TQ // 2))
            k_s[rows2, :] = as_u32(kv[:, 0:DH].astype(bf16))
            v_s[rows2, :] = as_u32(kv[:, DH:2 * DH].astype(bf16))
        qT_s[0] = (dot(wqT_s[...], xnT_s[0]) * (SCALE * LOG2E)).astype(bf16)

    def stage_dout(b):
        doutT = g_v[blk_rows(b), :].astype(f32).T
        doutT_s[...] = doutT
        doutb_s[...] = doutT.astype(bf16)

    def dhh_piece(j, r0, n):
        r = pl.ds(pl.multiple_of(j * FP + r0, 16), n)
        dhh_s[r, :] = dot(w2_v[r, :], doutb_s[...])

    par = i % 2
    common = (k_s, v_s, kT_s, vT_s)
    tail = (oT_s, dqT_s, dk_acc, dv_acc)

    @pl.when(i == 0)
    def _():
        attention(CFG_F, True, False, *common, qT_s.at[0], qT_s.at[1], doT_s, delta_s,
                  p0, p1, m0, m1, fin0, fin1, *tail)

    @pl.when(i == 0)
    def _late_weights():
        g_copy.wait()
        for c in late:
            c.wait()
        woT_s[...] = wo_v[...].T
        w1_s[...] = w1T_v[...].T
        w3_s[...] = w3T_v[...].T
        w2T_s[...] = w2_v[0:F, :].T
        stage_dout(0)
        dhh_s[...] = dot(w2_v[...], doutb_s[...])

    @pl.when(i == NB)
    def _early_grads():
        wo_v[...] = dwo_acc[...].astype(bf16)
        w1T_v[...] = dw1_acc[...].astype(bf16)
        w3T_v[...] = dw3_acc[...].astype(bf16)
        w2_v[0:F, :] = dw2_acc[...].astype(bf16)
        for c in grads:
            c.start()

    @pl.when(jnp.logical_and(jnp.logical_and(i > 0, i < NB), par == 0))
    def _():
        attention(CFG_M, True, True, *common, qT_s.at[0], qT_s.at[1], doT_s, delta_s,
                  p0, p1, m0, m1, fin0, fin1, *tail, filler=dhh_piece)

    @pl.when(jnp.logical_and(i < NB, par == 1))
    def _():
        attention(CFG_M, True, True, *common, qT_s.at[1], qT_s.at[0], doT_s, delta_s,
                  p1, p0, m1, m0, fin1, fin0, *tail, filler=dhh_piece)

    @pl.when(i == NB)
    def _():
        attention(CFG_B, False, True, *common, qT_s.at[0], qT_s.at[1], doT_s, delta_s,
                  p0, p1, m0, m1, fin0, fin1, *tail)

    def accumulate(ref, val):
        ref[...] = jnp.where(i > 0, ref[...], 0.0) + val

    def post_bwd(j):
        dqb = (dqT_s[...] * SCALE).astype(bf16)
        dxn = dot(wq_v[...], dqb)
        accumulate(dwq_acc, dot(xnT_s[j], dqb, NT))
        dxT_s[j] = dhT_s[...] + ln_bwd_cached(dxn, xT_s[j], st1_s[j, 0][0:1], st1_s[j, 1][0:1])

    @pl.when(i >= 2)
    def _():
        out_copy(i - 2).wait()

    @pl.when(i < NB)
    def _dense():
        doutT = doutT_s[...]
        doutb = doutb_s[...]
        xT = xT_s[i]
        oT = oT_s[DH:DH + D, :]
        ob = oT.astype(bf16)
        hT = xT + dot(woT_s[...], ob)
        dhh = dhh_s[0:F, :]
        post_bwd(jnp.maximum(i - 1, 0))
        xn2, rstd2 = ln_stats(hT)
        xn2b = xn2.astype(bf16)
        g = dot(w1T_v[...], xn2b)
        u = dot(w3T_v[...], xn2b)
        sig = jax.nn.sigmoid(g)
        silu = g * sig
        hh = (silu * u).astype(bf16)
        du = (dhh * silu).astype(bf16)
        dg = (dhh * u * (sig * (1.0 + g * (1.0 - sig)))).astype(bf16)
        outT = hT + dot(w2T_s[...], hh)
        out_v[par] = outT.T.astype(bf16)
        dxn2 = dot(w1_s[...], dg) + dot(w3_s[...], du)
        accumulate(dw2_acc, dot(hh, doutb, NT))
        accumulate(dw1_acc, dot(dg, xn2b, NT))
        accumulate(dw3_acc, dot(du, xn2b, NT))
        dhT = doutT + ln_bwd(dxn2, xn2, rstd2)
        dhT_s[...] = dhT
        dhb = dhT.astype(bf16)
        doT = dot(wo_v[...], dhb)
        qT_s[1 - par] = (dot(wqT_s[...], xnT_s[jnp.minimum(i + 1, NB - 1)])
                         * (SCALE * LOG2E)).astype(bf16)
        accumulate(dwo_acc, dot(ob, dhb, NT))
        doT_s[...] = doT
        delta = jnp.sum((doT * oT).reshape(H, DH, TQ), axis=1, keepdims=True)
        delta_s[...] = jnp.broadcast_to(delta, (H, 8, TQ))
        stage_dout(jnp.minimum(i + 1, NB - 1))

    @pl.when(i < NB)
    def _():
        out_copy(i).start()

    @pl.when(i == NB)
    def _epilogue():
        out_copy(NB - 1).wait()
        post_bwd(NB - 1)
        dwq_v[...] = dwq_acc[...].astype(bf16)
        dwq_copy.start()
        for b in range(NB):
            cols = slice(b * TQ, (b + 1) * TQ)
            dkv_s[b, 0:DH] = (dk_acc[:, cols] * (1.0 / LOG2E)).astype(bf16)
            dkv_s[b, DH:2 * DH] = dv_acc[:, cols].astype(bf16)
        wkvT = jnp.concatenate([wkT_v[...], wvT_v[...]], axis=0).astype(f32)
        wbar = jnp.sum(wkvT, axis=1, keepdims=True) * (1.0 / D)

        def chunk(c, dwkv):
            for bb in range(NB // XC):
                b = c * (NB // XC) + bb
                r0 = pl.multiple_of(b * TQ, TQ)
                dkv = dkv_s[b]
                d = dot(wkv_s[...], dkv)
                dkf = dkv.astype(f32)
                m1 = jnp.sum(wbar * dkf, axis=0, keepdims=True)
                m2 = jnp.sum(kvf_s[:, pl.ds(r0, TQ)] * dkf, axis=0, keepdims=True) * (1.0 / D)
                mu, rstd = st1_s[b, 0][0:1], st1_s[b, 1][0:1]
                bx = -(rstd * rstd) * m2
                dxT = dxT_s[b] + rstd * d + (bx * xT_s[b] + (-rstd * m1 - bx * mu))
                dx_v[pl.ds(r0, TQ), :] = dxT.T.astype(bf16)
                dwkv = dwkv + dot(dkv, xnT_s[b], NT)
            dx_copy(c).start()
            return dwkv
        dwkv = lax.fori_loop(0, XC, chunk, jnp.zeros((2 * DH, D), f32))
        dwkv_v[...] = dwkv.astype(bf16)
        dwk_copy.start()
        dwv_copy.start()
        for c in grads:
            c.wait()
        dwq_copy.wait()
        dwk_copy.wait()
        dwv_copy.wait()
        for c in range(XC):
            dx_copy(c).wait()


@jax.jit
def pallas_sequential_preLN__grouped_kv_mqa__glu_gated_swiglu__prompt_kernel(
    A_x, A_wq, A_wk, A_wv, A_wo, B_x, B_w1, B_w3, B_w2, grad_out):
    x = A_x.reshape(S, D)
    g = grad_out.reshape(S, D)
    blkspec = pl.BlockSpec((TQ, D), lambda i: (jnp.minimum(i, NB - 1), 0))
    anyspec = pl.BlockSpec(memory_space=pl.ANY)
    wshapes = [(D, D), (DH, D), (DH, D), (D, D), (F, D), (F, D), (F, D)]
    VM = pltpu.VMEM
    scratch = [
        VM((S, D), bf16), VM((S, D), bf16), VM((2, TQ, D), bf16), VM((D, D), bf16), VM((DH, D), bf16), VM((DH, D), bf16), VM((D, D), bf16),
        VM((F, D), bf16), VM((F, D), bf16), VM((FPAD, D), bf16),
        VM((S, D), bf16), VM((D, D), bf16), VM((2 * DH, D), bf16),
        VM((NB, D, TQ), f32), VM((NB, D, TQ), bf16), VM((NB, 2, 8, TQ), f32), VM((2 * DH, S), f32), VM((NB, 2 * DH, TQ), bf16),
        VM((D, D), bf16), VM((D, D), bf16), VM((D, F), bf16), VM((D, F), bf16), VM((D, F), bf16),
        VM((D, 2 * DH), bf16),
        VM((S // 2, DH), u32), VM((S // 2, DH), u32), VM((DH // 2, S), u32), VM((DH // 2, S), u32),
        VM((2, D, TQ), bf16), VM((D, TQ), f32), VM((H, 8, TQ), f32),
        VM((H + 1, S, TQ), bf16), VM((H + 1, S, TQ), bf16),
        VM((H, NC, 8, TQ), f32), VM((H, NC, 8, TQ), f32),
        VM((H + 1, 2, 8, TQ), f32), VM((H + 1, 2, 8, TQ), f32),
        VM((D + DH, TQ), f32), VM((D, TQ), f32), VM((D, TQ), f32),
        VM((FPAD, TQ), f32), VM((D, TQ), f32), VM((D, TQ), bf16),
        VM((DH, S), f32), VM((DH, S), f32), VM((NB, D, TQ), f32),
        VM((D, D), f32), VM((D, D), f32), VM((F, D), f32), VM((F, D), f32), VM((F, D), f32),
        pltpu.SemaphoreType.DMA((14,)),
    ]
    outs = pl.pallas_call(
        kernel,
        grid=(NB + 1,),
        in_specs=[anyspec] * (2 + len(wshapes)),
        out_specs=[anyspec] * (2 + len(wshapes)),
        out_shape=[jax.ShapeDtypeStruct((S, D), bf16), jax.ShapeDtypeStruct((S, D), bf16)]
        + [jax.ShapeDtypeStruct(s, bf16) for s in wshapes],
        scratch_shapes=scratch,
        compiler_params=pltpu.CompilerParams(
            dimension_semantics=("arbitrary",), vmem_limit_bytes=120 * 2**20),
        name="fused_block",
    )(x, g, A_wq, A_wk.T, A_wv.T, A_wo, B_w1.T, B_w3.T, B_w2)
    out, dx, dwq, dwkT, dwvT, dwo, dw1T, dw3T, dw2 = outs
    return (out.reshape(1, S, D), dx.reshape(1, S, D), dwq, dwkT.T, dwvT.T, dwo,
            dw1T.T, dw3T.T, dw2)
```
